```python
import jax
import jax.numpy as jnp

def _softmax(x, axis=-1):
    return jax.nn.softmax(x, axis=axis)

def _gelu(x):
    return jax.nn.gelu(x, approximate=True)

def _silu(x):
    return jax.nn.silu(x)

def _sigmoid(x):
    return jax.nn.sigmoid(x)

def _layernorm(x, axis=-1, eps=1e-05):
    m = jnp.mean(x, axis=axis, keepdims=True)
    v = jnp.var(x, axis=axis, keepdims=True)
    return (x - m) / jnp.sqrt(v + eps)

def _scatter_add(tgt, idx, src, axis=0):
    return tgt.at[idx].add(src)

def _segment_sum(src, seg, n):
    return jax.ops.segment_sum(src, seg, n)

class _Rng:

    def __init__(self, key):
        self._k = key

    def _next(self):
        self._k, sub = jax.random.split(self._k)
        return sub

    def normal(self, shape):
        return jax.random.normal(self._next(), shape, dtype=jnp.bfloat16)

    def randint(self, lo, hi, shape):
        return jax.random.randint(self._next(), shape, lo, hi, dtype=jnp.int32)

    def uniform(self, shape, lo=0.0, hi=1.0):
        return jax.random.uniform(self._next(), shape, jnp.bfloat16, lo, hi)

    def permutation(self, n):
        return jax.random.permutation(self._next(), n)
kernel_name = 'interleave_layers__linear_kernel_hedgehog__memory_aug_recurrent_mem_tr__prompt'

def setup_inputs():
    _rng = _Rng(jax.random.key(int.from_bytes(__import__("os").urandom(4), "little")))
    _w = lambda a: (lambda t: t.astype(jnp.bfloat16) if jnp.issubdtype(t.dtype, jnp.floating) else t)(jnp.asarray(a))

    def _A_setup():
        B, S, D, H = (1, 2048, 640, 32)
        Dh = D // H
        return {'x': _w((lambda *s: _rng.normal(s) * 0.05)(B, S, D)), 'wqkv': _w((lambda *s: _rng.normal(s) * 0.05)(D, 3 * D)), 'w_phi': _w((lambda *s: _rng.normal(s) * 0.05)(H, Dh, Dh) * Dh ** (-0.5)), 'wo': _w((lambda *s: _rng.normal(s) * 0.05)(D, D))}
    _A_in = _A_setup()

    def _B_setup():
        B, S, Dm = (1, 2048, 640)
        H, Dh = (32, 192)
        M, seg = (8, 32)
        seg = min(seg, S)
        S = S // seg * seg
        return {'x': _w((lambda *s: _rng.normal(s) * 0.05)(B, S, Dm)), 'mem0': _w((lambda *s: _rng.normal(s) * 0.05)(B, M, Dm)), 'Wq': _w((lambda *s: _rng.normal(s) * 0.05)(Dm, H, Dh) * Dm ** (-0.5)), 'Wk': _w((lambda *s: _rng.normal(s) * 0.05)(Dm, H, Dh) * Dm ** (-0.5)), 'Wv': _w((lambda *s: _rng.normal(s) * 0.05)(Dm, H, Dh) * Dm ** (-0.5)), 'Wo': _w((lambda *s: _rng.normal(s) * 0.05)(H, Dh, Dm) * (H * Dh) ** (-0.5)), 'seg_len': seg}
    _B_in = _B_setup()
    return {'A_x': _A_in['x'], 'A_wqkv': _A_in['wqkv'], 'A_w_phi': _A_in['w_phi'], 'A_wo': _A_in['wo'], 'B_x': _B_in['x'], 'B_mem0': _B_in['mem0'], 'B_Wq': _B_in['Wq'], 'B_Wk': _B_in['Wk'], 'B_Wv': _B_in['Wv'], 'B_Wo': _B_in['Wo'], 'B_seg_len': _B_in['seg_len']}

def reference(A_x, A_wqkv, A_w_phi, A_wo, B_x, B_mem0, B_Wq, B_Wk, B_Wv, B_Wo, B_seg_len):

    def _A_ref(x, wqkv, w_phi, wo):
        B, S, D = x.shape
        H = 32
        Dh = D // H
        qkv = (lambda x, *d: x.transpose(*d))((x @ wqkv).reshape(B, S, 3, H, Dh), 2, 0, 3, 1, 4)
        q, k, v = (qkv[0], qkv[1], qkv[2])
        pq = jnp.einsum('bhsd,hdf->bhsf', q, w_phi)
        pk = jnp.einsum('bhsd,hdf->bhsf', k, w_phi)
        phi_q = jnp.concatenate([_softmax(pq, axis=-1), _softmax(-pq, axis=-1)], axis=-1)
        phi_k = jnp.concatenate([_softmax(pk, axis=-1), _softmax(-pk, axis=-1)], axis=-1)
        kv = jnp.einsum('bhsf,bhsd->bhfd', phi_k, v)
        z = jnp.einsum('bhsf->bhf', phi_k)
        num = jnp.einsum('bhqf,bhfd->bhqd', phi_q, kv)
        den = jnp.einsum('bhqf,bhf->bhq', phi_q, z)[..., None] + 1e-06
        o = num / den
        return (lambda x, *d: x.transpose(*d))(o, 0, 2, 1, 3).reshape(B, S, D) @ wo

    def _B_ref(x, mem0, Wq, Wk, Wv, Wo, seg_len):
        B, S, Dm = x.shape
        H, Dh = (Wq.shape[1], Wq.shape[2])
        M = mem0.shape[1]
        scale = Dh ** (-0.5)
        n_seg = S // seg_len
        L = M + seg_len
        idx = jnp.arange(L)
        mask = (idx[:, None] < M) | (idx[:, None] >= idx[None, :])
        mem = mem0
        outs = []
        for s in range(n_seg):
            xs = x[:, s * seg_len:(s + 1) * seg_len, :].copy()
            h = jnp.concatenate([mem, xs], axis=1)
            q = jnp.einsum('btd,dhe->bhte', h, Wq)
            k = jnp.einsum('btd,dhe->bhte', h, Wk)
            v = jnp.einsum('btd,dhe->bhte', h, Wv)
            scores = jnp.einsum('bhqe,bhke->bhqk', q, k) * scale
            scores = jnp.where(mask[None, None], scores, -1000000000.0)
            p = _softmax(scores, axis=-1)
            o = jnp.einsum('bhqk,bhke->bhqe', p, v)
            o = jnp.einsum('bhte,hed->btd', o, Wo)
            mem = o[:, :M, :].copy()
            outs.append(o[:, M:, :])
        return jnp.concatenate(outs, axis=1)
    x = A_x
    x = x + _A_ref(_layernorm(x, axis=-1), A_wqkv, A_w_phi, A_wo)
    x = x + _B_ref(_layernorm(x, axis=-1), B_mem0, B_Wq, B_Wk, B_Wv, B_Wo, B_seg_len)
    x = x + _A_ref(_layernorm(x, axis=-1), A_wqkv, A_w_phi, A_wo)
    x = x + _B_ref(_layernorm(x, axis=-1), B_mem0, B_Wq, B_Wk, B_Wv, B_Wo, B_seg_len)
    return x
```

```python
import functools
import jax
import jax.numpy as jnp
from jax import lax
import jax.experimental.pallas as pl
import jax.experimental.pallas.tpu as pltpu

F32, BF = jnp.float32, jnp.bfloat16
NT = (((1,), (1,)), ((), ()))


def _dot(a, b):
    return jnp.dot(a, b, preferred_element_type=F32)


def _ln(x):
    m = jnp.mean(x, axis=-1, keepdims=True)
    c = x - m
    v = jnp.mean(c * c, axis=-1, keepdims=True)
    return c * lax.rsqrt(v + 1e-5)


def _kernel(x_ref, wqkv_ref, phi_ref, wo_ref, mem0_ref, wq_h, wk_h, wv_h, wo_h,
            o_ref, xs, wq, wk, wv, wob, wfq, wfk, pq_s, kv_s, sems, *, seg):
    S, D = x_ref.shape
    H, Dh = 32, D // 32
    M = mem0_ref.shape[0]
    L = M + seg
    TB = 256
    E = 192
    cps = [pltpu.make_async_copy(s, d, sems.at[i]) for i, (s, d) in
           enumerate(((wq_h, wq), (wk_h, wk), (wv_h, wv), (wo_h, wob)))]
    for c in cps:
        c.start()

    r = lax.broadcasted_iota(jnp.int32, (D, D), 0)
    c = lax.broadcasted_iota(jnp.int32, (D, D), 1)
    bd = jnp.where(r // Dh == c % H, phi_ref[...].astype(F32), 0.0).astype(BF)
    wfq[...] = _dot(wqkv_ref[:, 0:D], bd).T.astype(BF)
    wfk[...] = _dot(wqkv_ref[:, D:2 * D], bd).T.astype(BF)
    xs[...] = x_ref[...].astype(F32)

    def feat(p):
        sl = [p[f * H:(f + 1) * H] for f in range(Dh)]
        mx = functools.reduce(jnp.maximum, sl)
        mn = functools.reduce(jnp.minimum, sl)
        a = [jnp.exp(s - mx) for s in sl]
        b = [jnp.exp(mn - s) for s in sl]
        ia = 1.0 / functools.reduce(jnp.add, a)
        ib = 1.0 / functools.reduce(jnp.add, b)
        return jnp.concatenate([t * ia for t in a] + [t * ib for t in b], axis=0).astype(BF)

    def layer_a():
        kv_s[...] = jnp.zeros_like(kv_s)

        def p1(i, _):
            o = pl.multiple_of(i * TB, TB)
            xn = _ln(xs[pl.ds(o, TB), :]).astype(BF)
            pq_s[:, pl.ds(o, TB)] = feat(lax.dot_general(wfq[...], xn, NT, preferred_element_type=F32))
            pk = feat(lax.dot_general(wfk[...], xn, NT, preferred_element_type=F32))
            v = _dot(xn, wqkv_ref[:, 2 * D:3 * D]).astype(BF)
            v = jnp.concatenate([v, jnp.ones((TB, 128), BF)], axis=1)
            kv_s[...] += _dot(pk, v)
            return 0
        lax.fori_loop(0, S // TB, p1, 0)
        rr = lax.broadcasted_iota(jnp.int32, (2 * D, D), 0)
        cc = lax.broadcasted_iota(jnp.int32, (2 * D, D), 1)
        kvm = jnp.where(rr % H == cc // Dh, kv_s[:, 0:D], 0.0).astype(BF)
        mt = _dot(kvm, wo_ref[...]).T.astype(BF)
        z = kv_s[:, D:D + 128]
        z = jnp.concatenate([z] * (TB // 128), axis=1)

        def p2(i, _):
            o = pl.multiple_of(i * TB, TB)
            p = pq_s[:, pl.ds(o, TB)].astype(F32)
            pz = p * z
            den = functools.reduce(jnp.add, [pz[f * H:(f + 1) * H] for f in range(2 * Dh)])
            inv = 1.0 / (den + 1e-6)
            pn = (p * jnp.concatenate([inv] * (2 * Dh), axis=0)).astype(BF)
            xs[pl.ds(o, TB), :] += _dot(mt, pn).T
            return 0
        lax.fori_loop(0, S // TB, p2, 0)

    def layer_b():
        P = 2 * E
        lane = lax.broadcasted_iota(jnp.int32, (L, P), 1)
        ma = lane < E
        qi = lax.broadcasted_iota(jnp.int32, (L, 2 * L), 0)
        ki = lax.broadcasted_iota(jnp.int32, (L, 2 * L), 1)
        first = ki < L
        ok = (qi < M) | (qi >= jnp.where(first, ki, ki - L))
        scale = E ** -0.5

        def step(s, mem):
            o = pl.multiple_of(s * seg, seg)
            xb = xs[pl.ds(o, seg), :]
            h = jnp.concatenate([mem, _ln(xb)], axis=0).astype(BF)
            q = _dot(h, wq[...])
            k = _dot(h, wk[...])
            v = _dot(h, wv[...])
            outs = []
            for j in range(H // 2):
                qp, kp, vp = (t[:, j * P:(j + 1) * P] for t in (q, k, v))
                k2 = jnp.concatenate([jnp.where(ma, kp, 0.0), jnp.where(ma, 0.0, kp)], axis=0).astype(BF)
                v2 = jnp.concatenate([jnp.where(ma, vp, 0.0), jnp.where(ma, 0.0, vp)], axis=0).astype(BF)
                sc = lax.dot_general(qp.astype(BF), k2, NT, preferred_element_type=F32) * scale
                sc = jnp.where(ok, sc, -1e9)
                m1 = jnp.max(jnp.where(first, sc, -jnp.inf), axis=1, keepdims=True)
                m2 = jnp.max(jnp.where(first, -jnp.inf, sc), axis=1, keepdims=True)
                e = jnp.exp(sc - jnp.where(first, m1, m2))
                s1 = jnp.sum(jnp.where(first, e, 0.0), axis=1, keepdims=True)
                s2 = jnp.sum(jnp.where(first, 0.0, e), axis=1, keepdims=True)
                p = e * jnp.where(first, 1.0 / s1, 1.0 / s2)
                outs.append(_dot(p.astype(BF), v2).astype(BF))
            y = _dot(jnp.concatenate(outs, axis=1), wob[...])
            xs[pl.ds(o, seg), :] = xb + y[M:]
            return y[:M]
        lax.fori_loop(0, S // seg, step, mem0_ref[...].astype(F32))

    def layer(i, _):
        layer_a()

        @pl.when(i == 0)
        def _():
            for c in cps:
                c.wait()
        layer_b()
        return 0
    lax.fori_loop(0, 2, layer, 0)
    o_ref[...] = xs[...].astype(o_ref.dtype)


@functools.partial(jax.jit, static_argnames=("B_seg_len",))
def pallas_interleave_layers__linear_kernel_hedgehog__memory_aug_recurrent_mem_tr__prompt_kernel(
        A_x, A_wqkv, A_w_phi, A_wo, B_x, B_mem0, B_Wq, B_Wk, B_Wv, B_Wo, B_seg_len):
    _, S, D = A_x.shape
    H, Dh, _ = A_w_phi.shape
    HE = B_Wq.shape[1] * B_Wq.shape[2]
    phi = jnp.broadcast_to(A_w_phi.reshape(D, Dh, 1), (D, Dh, H)).reshape(D, D)
    vm = pl.BlockSpec(memory_space=pltpu.VMEM)
    an = pl.BlockSpec(memory_space=pl.ANY)
    out = pl.pallas_call(
        functools.partial(_kernel, seg=int(B_seg_len)),
        in_specs=[vm] * 5 + [an] * 4,
        out_specs=vm,
        out_shape=jax.ShapeDtypeStruct((S, D), A_x.dtype),
        scratch_shapes=[pltpu.VMEM((S, D), F32)] + [pltpu.VMEM((D, HE), BF)] * 3
        + [pltpu.VMEM((HE, D), BF), pltpu.VMEM((D, D), BF), pltpu.VMEM((D, D), BF),
           pltpu.VMEM((2 * D, S), BF), pltpu.VMEM((2 * D, D + 128), F32),
           pltpu.SemaphoreType.DMA((4,))],
        compiler_params=pltpu.CompilerParams(vmem_limit_bytes=100 * 2**20),
    )(A_x[0], A_wqkv, phi, A_wo, B_mem0[0], B_Wq.reshape(D, HE), B_Wk.reshape(D, HE),
      B_Wv.reshape(D, HE), B_Wo.reshape(HE, D))
    return out[None]
```
